```python
import os as _os
_os.environ.setdefault('JAX_PLATFORMS', 'cpu')
import jax
import jax.numpy as jnp

def _softmax(x, axis=-1):
    return jax.nn.softmax(x, axis=axis)

def _gelu(x):
    return jax.nn.gelu(x, approximate=True)

def _silu(x):
    return jax.nn.silu(x)

def _sigmoid(x):
    return jax.nn.sigmoid(x)

def _layernorm(x, axis=-1, eps=1e-05):
    m = jnp.mean(x, axis=axis, keepdims=True)
    v = jnp.var(x, axis=axis, keepdims=True)
    return (x - m) / jnp.sqrt(v + eps)

def _scatter_add(tgt, idx, src, axis=0):
    return tgt.at[idx].add(src)

def _segment_sum(src, seg, n):
    return jax.ops.segment_sum(src, seg, n)

class _Rng:

    def __init__(self, key):
        self._k = key

    def _next(self):
        self._k, sub = jax.random.split(self._k)
        return sub

    def normal(self, shape):
        return jax.random.normal(self._next(), shape, dtype=jnp.bfloat16)

    def randint(self, lo, hi, shape):
        return jax.random.randint(self._next(), shape, lo, hi, dtype=jnp.int32)

    def uniform(self, shape, lo=0.0, hi=1.0):
        return jax.random.uniform(self._next(), shape, jnp.bfloat16, lo, hi)

    def permutation(self, n):
        return jax.random.permutation(self._next(), n)
kernel_name = 'standalone__conformer_conv_module__speech'

def setup_inputs():
    _rng = _Rng(jax.random.key(int.from_bytes(__import__("os").urandom(4), "little")))
    _w = lambda a: (lambda t: t.astype(jnp.bfloat16) if jnp.issubdtype(t.dtype, jnp.floating) else t)(jnp.asarray(a))
    B, T, D, K = (2, 4000, 512, 15)
    return {'x': _w((lambda *s: _rng.normal(s) * 0.2)(B, T, D)), 'w_pw1': _w((lambda *s: _rng.normal(s) * 0.2)(D, 2 * D)), 'dw': _w((lambda *s: _rng.normal(s) * 0.05)(K, D)), 'w_pw2': _w((lambda *s: _rng.normal(s) * 0.05)(D, D))}

def reference(x, w_pw1, dw, w_pw2):
    B, T, D = x.shape
    K = dw.shape[0]
    h = x @ w_pw1
    a, b = (h[..., :D].copy(), h[..., D:].copy())
    h = a * _sigmoid(b)
    pad = K // 2
    hp = jnp.pad(h, ((0, 0), (pad, pad), (0, 0)))
    out = jnp.zeros_like(h)
    for i in range(K):
        out = out + hp[:, i:i + T, :] * dw[i][None, None, :]
    return _silu(out) @ w_pw2
```

```python
import bisect
import functools

import jax
import jax.numpy as jnp
from jax import lax
import jax.experimental.pallas as pl
import jax.experimental.pallas.tpu as pltpu

LANES = 128
SUBLANES = 8
ROW_TILE = 16
HALO = SUBLANES


def _prefix_sums(sizes):
    return [sum(sizes[:i]) for i in range(len(sizes) + 1)]


def _plan_chunks(T):
    head = [288, 256]
    tiles = (T - sum(head)) // ROW_TILE
    count = max(2, round(tiles / 27))
    return head + [
        (tiles // count + (i < tiles % count)) * ROW_TILE for i in range(count)
    ]


def _make_kernel(B, T, D, K):
    NJ = D // LANES
    pad = K // 2
    chunks = _plan_chunks(T)
    top = _prefix_sums(chunks)
    conv_top = [0] + [t - ROW_TILE for t in top[1:-1]] + [T]
    out_top = [0] + conv_top[2:-1] + [T - LANES, T]
    conv_delay, conv_step = 64, 16
    out_lag = 2

    def kernel(x_hbm, w1_hbm, dw_hbm, w2_hbm, o_hbm,
               x_buf, w_buf, dw_buf, taps, h_buf, s_buf, o_buf,
               x_sem, w_sem, o_sem):

        def column(j):
            return pl.ds(j * LANES, LANES)

        def w1_copy(p):
            t = p // 2 + (NJ if p % 2 == 0 else 0)
            return pltpu.make_async_copy(
                w1_hbm.at[:, column(t)], w_buf.at[t], w_sem.at[max(p - 1, 0)])

        def w2_copy(j):
            return pltpu.make_async_copy(
                w2_hbm.at[:, column(j)], w_buf.at[2 * NJ + j], w_sem.at[0])

        def x_copy(b, i):
            rows = pl.ds(top[i], chunks[i])
            return pltpu.make_async_copy(
                x_hbm.at[b, rows], x_buf.at[rows], x_sem)

        dw_copy = pltpu.make_async_copy(dw_hbm, dw_buf, w_sem.at[0])

        x_copy(0, 0).start()
        dw_copy.start()
        for p in range(2 * NJ):
            w1_copy(p).start(priority=int(p >= 2))
        zeros = jnp.zeros((NJ, HALO, LANES), jnp.float32)
        h_buf[:, pl.ds(0, HALO), :] = zeros
        h_buf[:, pl.ds(HALO + T, HALO), :] = zeros

        def sequence(b, carry):
            on_first = pl.when(b == 0)
            results, result_top = [], [0]
            pending = []
            last_anchor = [0]

            def for_this_sequence(fn):
                for k in range(B):
                    pl.when(b == k)(functools.partial(fn, k))

            def matmul(lhs, tile):
                y = jnp.dot(lhs, w_buf[tile],
                            preferred_element_type=jnp.float32)
                results.append(y)
                result_top.append(result_top[-1] + y.shape[0])
                return y

            def result_rows(pos):
                pos = min(pos, result_top[-1] - SUBLANES)
                n = bisect.bisect_right(result_top, pos) - 1
                pos -= result_top[n]
                return results[n][pos:pos + SUBLANES]

            def copies_before(i, p):
                if p == 0:
                    x_copy(b, i).wait()
                if p == 1 and i + 1 < len(chunks):
                    for_this_sequence(
                        lambda k: x_copy(k, i + 1).start(priority=1))
                if p == 1 and i + 1 == len(chunks):
                    for k in range(1, B):
                        pl.when(b == k - 1)(
                            lambda k=k: x_copy(k, 0).start(priority=1))
                if (i, p) == (0, 0):
                    @on_first
                    def _():
                        dw_copy.wait()
                        w1_copy(0).wait()
                        w1_copy(1).wait()

                    taps[...] = dw_buf[...].astype(jnp.float32) * 0.25
                if i == 0 and p >= 2:
                    on_first(lambda: w1_copy(p).wait())
                if (i, p) == (1, 2):
                    @on_first
                    def _():
                        for j in range(NJ):
                            w2_copy(j).start(priority=1)

            def glu(i, j):
                rows = pl.ds(top[i], chunks[i])
                h_rows = pl.ds(HALO + top[i], chunks[i])
                copies_before(i, 2 * j)
                gate = matmul(x_buf[rows, :], NJ + j)
                h_buf[j, h_rows, :] = jnp.tanh(gate * 0.5)
                convolve_pending(0)
                copies_before(i, 2 * j + 1)
                base = result_top[-1]
                value = matmul(x_buf[rows, :], j)
                h_buf[j, h_rows, :] = value + value * h_buf[j, h_rows, :]
                anchors = []
                for t in range(conv_top[i], conv_top[i + 1] + SUBLANES,
                               SUBLANES):
                    last_anchor[0] = max(
                        base + max(t - top[i], 0) + conv_delay,
                        last_anchor[0] + conv_step)
                    anchors.append(last_anchor[0])
                last_anchor[0] -= conv_step
                pending.append((i, j, anchors))
                convolve_pending(0)

            def convolve(i, j, anchors):
                r, c = conv_top[i], conv_top[i + 1] - conv_top[i]
                w = [taps[k:k + 1, column(j)] for k in range(K)]
                low = high = None
                for k in range(SUBLANES):
                    paired = k + SUBLANES < K
                    h = h_buf[j, pl.ds(HALO - pad + r + k,
                                       c + SUBLANES * paired), :]
                    if k == 0:
                        lane = lax.broadcasted_iota(jnp.int32, h.shape, 1)
                        later = jnp.concatenate(
                            [result_rows(a) for a in anchors], axis=0)
                        h = jnp.where(lane == LANES + b, later, h)
                    if paired:
                        term = h[SUBLANES:] * w[k + SUBLANES]
                        high = term if high is None else high + term
                    term = h[:c] * w[k]
                    low = term if low is None else low + term
                y = low + high
                s_buf[j, pl.ds(r, c), :] = (
                    y + y * jnp.tanh(y)).astype(s_buf.dtype)

            def convolve_pending(rows_needed):
                while pending and (conv_top[pending[0][0]] < rows_needed
                                   or pending[0][2][-1] < result_top[-1]):
                    convolve(*pending.pop(0))

            def project(i, j):
                convolve_pending(out_top[i + 1])
                rows = pl.ds(out_top[i], out_top[i + 1] - out_top[i])
                if (i, j) == (0, 0):
                    @on_first
                    def _():
                        for t in range(NJ):
                            w2_copy(t).wait()
                s = jnp.concatenate(
                    [s_buf[t, rows, :] for t in range(NJ)], axis=1)
                o_buf[b, j, rows, :] = matmul(s, 2 * NJ + j).astype(
                    o_buf.dtype)
                for_this_sequence(lambda k: pltpu.make_async_copy(
                    o_buf.at[k, j, rows], o_hbm.at[k, rows, column(j)],
                    o_sem).start())
                convolve_pending(0)

            todo = [
                (bisect.bisect_left(conv_top, out_top[i + 1]) * NJ - 1
                 + out_lag + j, i, j)
                for i in range(len(out_top) - 1) for j in range(NJ)
            ]
            for q in range(len(chunks) * NJ):
                glu(q // NJ, q % NJ)
                if todo[0][0] <= q:
                    project(*todo.pop(0)[1:])
            for _, i, j in todo:
                project(i, j)
            return carry

        lax.fori_loop(0, B, sequence, 0)
        pltpu.make_async_copy(o_buf, o_buf, o_sem).wait()

    return kernel


@jax.jit
def pallas_standalone__conformer_conv_module__speech_kernel(
    x: jax.Array,
    w_pw1: jax.Array,
    dw: jax.Array,
    w_pw2: jax.Array,
):
    B, T, D = x.shape
    K = dw.shape[0]
    NJ = D // LANES
    assert D % LANES == 0 and NJ >= 2 and T % ROW_TILE == 0 and T >= 1024
    assert K % 2 == 1 and SUBLANES < K < 2 * SUBLANES

    return pl.pallas_call(
        _make_kernel(B, T, D, K),
        out_shape=jax.ShapeDtypeStruct((B, T, D), x.dtype),
        in_specs=[pl.BlockSpec(memory_space=pl.ANY)] * 4,
        out_specs=pl.BlockSpec(memory_space=pl.ANY),
        scratch_shapes=[
            pltpu.VMEM((T, D), x.dtype),
            pltpu.VMEM((3 * NJ, D, LANES), w_pw1.dtype),
            pltpu.VMEM((K, D), dw.dtype),
            pltpu.VMEM((K, D), jnp.float32),
            pltpu.VMEM((NJ, T + 2 * HALO, LANES), jnp.float32),
            pltpu.VMEM((NJ, T, LANES), x.dtype),
            pltpu.VMEM((B, NJ, T, LANES), x.dtype),
            pltpu.SemaphoreType.DMA(()),
            pltpu.SemaphoreType.DMA((2 * NJ - 1,)),
            pltpu.SemaphoreType.DMA(()),
        ],
        compiler_params=pltpu.CompilerParams(
            vmem_limit_bytes=64 * 1024 * 1024,
            flags={"XLA_TPU_RESCHEDULE_DMA_DONES": True},
        ),
        name="conformer_conv",
    )(x, w_pw1, dw, w_pw2)
```
